```python
import os as _os
_os.environ.setdefault("JAX_PLATFORMS", "cpu")
import jax
import jax.numpy as jnp

def _softmax(x, axis=-1):
    return jax.nn.softmax(x, axis=axis)
def _gelu(x):
    return jax.nn.gelu(x, approximate=True)
def _silu(x):
    return jax.nn.silu(x)
def _sigmoid(x):
    return jax.nn.sigmoid(x)
def _layernorm(x, axis=-1, eps=1e-5):
    m = jnp.mean(x, axis=axis, keepdims=True)
    v = jnp.var(x, axis=axis, keepdims=True)
    return (x - m) / jnp.sqrt(v + eps)
def _scatter_add(tgt, idx, src, axis=0):
    return tgt.at[idx].add(src)
def _segment_sum(src, seg, n):
    return jax.ops.segment_sum(src, seg, n)
class _Rng:
    def __init__(self, key):
        self._k = key
    def _next(self):
        self._k, sub = jax.random.split(self._k)
        return sub
    def normal(self, shape):
        return jax.random.normal(self._next(), shape, dtype=jnp.bfloat16)
    def randint(self, lo, hi, shape):
        return jax.random.randint(self._next(), shape, lo, hi, dtype=jnp.int32)
    def uniform(self, shape, lo=0.0, hi=1.0):
        return jax.random.uniform(self._next(), shape, jnp.bfloat16, lo, hi)
    def permutation(self, n):
        return jax.random.permutation(self._next(), n)


kernel_name = 'parallel_sum__sliding_local_dilated__glu_gated_geglu__prompt'

def setup_inputs():
    _rng = _Rng(jax.random.key(int.from_bytes(__import__("os").urandom(4), "little")))
    _w = (lambda a: (lambda t: t.astype(jnp.bfloat16) if jnp.issubdtype(t.dtype, jnp.floating) else t)(jnp.asarray(a)))
    def _A_setup():
        B, S, D = 1, 2048, 512
        return {
            "x": _w((lambda *s: _rng.normal(s) * 0.05)(B, S, D)),
            "wqkv": _w((lambda *s: _rng.normal(s) * 0.05)(D, 3 * D)),
            "wo": _w((lambda *s: _rng.normal(s) * 0.05)(D, D)),
        }
    _A_in = _A_setup()

    def _B_setup():
        B, S, Dm, Df = 1, 2048, 512, 1376
        return {
            "x": _w((lambda *s: _rng.normal(s) * 0.05)(B, S, Dm)),
            "w_gate": _w((lambda *s: _rng.normal(s) * 0.1)(Dm, Df) * (Dm ** -0.5)),
            "w_up": _w((lambda *s: _rng.normal(s) * 0.1)(Dm, Df) * (Dm ** -0.5)),
            "w_down": _w((lambda *s: _rng.normal(s) * 0.1)(Df, Dm) * (Df ** -0.5)),
        }
    _B_in = _B_setup()

    return {
        "A_x": _A_in["x"],
        "A_wqkv": _A_in["wqkv"],
        "A_wo": _A_in["wo"],
        "B_x": _B_in["x"],
        "B_w_gate": _B_in["w_gate"],
        "B_w_up": _B_in["w_up"],
        "B_w_down": _B_in["w_down"],
    }

def reference(A_x, A_wqkv, A_wo, B_x, B_w_gate, B_w_up, B_w_down):
    def _A_ref(x, wqkv, wo):
        B, S, D = x.shape
        H = 32; Dh = D // H
        W, dil = 8, 2
        qkv = (lambda x, *d: x.transpose(*d))((x @ wqkv).reshape(B, S, 3, H, Dh), 2, 0, 3, 1, 4)
        q, k, v = qkv[0], qkv[1], qkv[2]
        scale = Dh ** -0.5
        pos = jnp.arange(S)
        off = jnp.arange(W) * dil
        idx = pos[:, None] - off[None, :]
        mask = idx >= 0
        idx_c = jnp.where(mask, idx, 0).reshape(-1)
        kg = k[:, :, idx_c, :].reshape(B, H, S, W, Dh)
        vg = v[:, :, idx_c, :].reshape(B, H, S, W, Dh)
        logits = jnp.einsum("bhsd,bhswd->bhsw", q, kg) * scale
        logits = jnp.where(mask[None, None, :, :], logits, -1e9)
        attn = _softmax(logits, axis=-1)
        o = jnp.einsum("bhsw,bhswd->bhsd", attn, vg)
        return (lambda x, *d: x.transpose(*d))(o, 0, 2, 1, 3).reshape(B, S, D) @ wo

    def _B_ref(x, w_gate, w_up, w_down):
        g = jnp.einsum("bsd,df->bsf", x, w_gate)
        u = jnp.einsum("bsd,df->bsf", x, w_up)
        h = _gelu(g) * u
        return jnp.einsum("bsf,fd->bsd", h, w_down)

    x = A_x
    xn = _layernorm(x, axis=-1)
    return x + _A_ref(xn, A_wqkv, A_wo) + _B_ref(xn, B_w_gate, B_w_up, B_w_down)
```

```python
import functools

import jax
import jax.numpy as jnp
import jax.experimental.pallas as pl
import jax.experimental.pallas.tpu as pltpu

S = 2048
D = 512
H = 32
DH = 16
W = 8
DIL = 2
DF = 1376
HALO = 16
TM = 256
EPS = 1e-5
NEG = -1e9
SCALE = DH ** -0.5
GELU_C = 0.7978845608028654


def _kernel(x_ref, wqkv_ref, wo_ref, wg_ref, wu_ref, wd_ref, o_ref, kbuf, vbuf):
    i = pl.program_id(0)
    f32 = jnp.float32
    bf16 = jnp.bfloat16

    x = x_ref[...].astype(f32)
    m = jnp.mean(x, axis=-1, keepdims=True)
    xc = x - m
    var = jnp.mean(xc * xc, axis=-1, keepdims=True)
    xn = (xc * jax.lax.rsqrt(var + EPS)).astype(bf16)

    qkv = jnp.dot(xn, wqkv_ref[...], preferred_element_type=f32)
    q = qkv[:, :D] * SCALE

    @pl.when(i == 0)
    def _():
        kbuf[0:HALO, :] = jnp.zeros((HALO, D), f32)
        vbuf[0:HALO, :] = jnp.zeros((HALO, D), f32)

    kbuf[HALO:, :] = qkv[:, D:2 * D]
    vbuf[HALO:, :] = qkv[:, 2 * D:]

    row = i * TM + jax.lax.broadcasted_iota(jnp.int32, (TM, 128), 0)
    logits = []
    for w in range(W):
        ks = kbuf[HALO - DIL * w: HALO - DIL * w + TM, :]
        p = q * ks
        p = (p[:, 0:128] + p[:, 128:256]) + (p[:, 256:384] + p[:, 384:512])
        p = p + pltpu.roll(p, 32, 1)
        p = p + pltpu.roll(p, 64, 1)
        if w > 0:
            p = jnp.where(row >= DIL * w, p, NEG)
        logits.append(p)
    mx = logits[0]
    for w in range(1, W):
        mx = jnp.maximum(mx, logits[w])
    es = [jnp.exp(l - mx) for l in logits]
    den = es[0]
    for w in range(1, W):
        den = den + es[w]
    inv = 1.0 / den
    acc = [None] * 4
    for w in range(W):
        a = es[w] * inv
        vs = vbuf[HALO - DIL * w: HALO - DIL * w + TM, :]
        for j in range(4):
            t = a * vs[:, 128 * j:128 * (j + 1)]
            acc[j] = t if acc[j] is None else acc[j] + t
    o = jnp.concatenate(acc, axis=-1).astype(bf16)

    kbuf[0:HALO, :] = kbuf[TM:TM + HALO, :]
    vbuf[0:HALO, :] = vbuf[TM:TM + HALO, :]

    ya = jnp.dot(o, wo_ref[...], preferred_element_type=f32)

    g = jnp.dot(xn, wg_ref[...], preferred_element_type=f32)
    u = jnp.dot(xn, wu_ref[...], preferred_element_type=f32)
    gl = 0.5 * g * (1.0 + jnp.tanh(GELU_C * (g + 0.044715 * (g * g * g))))
    h = (gl * u).astype(bf16)
    yb = jnp.dot(h, wd_ref[...], preferred_element_type=f32)

    o_ref[...] = (x + ya + yb).astype(o_ref.dtype)


@jax.jit
def pallas_parallel_sum__sliding_local_dilated__glu_gated_geglu__prompt_kernel(
    A_x: jax.Array,
    A_wqkv: jax.Array,
    A_wo: jax.Array,
    B_x: jax.Array,
    B_w_gate: jax.Array,
    B_w_up: jax.Array,
    B_w_down: jax.Array,
):
    x = A_x.reshape(S, D)
    wqkv = A_wqkv.reshape(D, 3, H, DH).transpose(0, 1, 3, 2).reshape(D, 3 * D)
    wo = A_wo.reshape(H, DH, D).transpose(1, 0, 2).reshape(D, D)

    const = lambda i: (0, 0)
    out = pl.pallas_call(
        _kernel,
        grid=(S // TM,),
        in_specs=[
            pl.BlockSpec((TM, D), lambda i: (i, 0)),
            pl.BlockSpec((D, 3 * D), const),
            pl.BlockSpec((D, D), const),
            pl.BlockSpec((D, DF), const),
            pl.BlockSpec((D, DF), const),
            pl.BlockSpec((DF, D), const),
        ],
        out_specs=pl.BlockSpec((TM, D), lambda i: (i, 0)),
        out_shape=jax.ShapeDtypeStruct((S, D), jnp.bfloat16),
        scratch_shapes=[
            pltpu.VMEM((TM + HALO, D), jnp.float32),
            pltpu.VMEM((TM + HALO, D), jnp.float32),
        ],
        compiler_params=pltpu.CompilerParams(
            dimension_semantics=("arbitrary",),
            vmem_limit_bytes=96 * 1024 * 1024,
        ),
    )(x, wqkv, wo, B_w_gate, B_w_up, B_w_down)
    return out.reshape(1, S, D)
```

```python
import functools

import jax
import jax.numpy as jnp
import jax.experimental.pallas as pl
import jax.experimental.pallas.tpu as pltpu

S = 2048
D = 512
H = 32
DH = 16
W = 8
DIL = 2
DF = 1376
HALO = 16
TM = 512
NSTEP = S // TM
RC = 16
EPS = 1e-5
LOG2E = 1.4426950408889634
NEG = -1e9 * LOG2E
SCALE = DH ** -0.5 * LOG2E
GELU_C = 0.7978845608028654
NT = (((1,), (1,)), ((), ()))
GA, GB = 384, 896


def _kernel(x_hbm, wqkv_hbm, wo_hbm, wg_hbm, wu_hbm, wd_hbm, o_ref,
            xbuf, wqkv_raw, wo_raw, wg_v, wu_v, wd_v, wqkvT, wo_p, tbuf, tbuf2,
            csbuf, qbuf, kbuf, vbuf, obuf, sems, xsems):
    i = pl.program_id(0)
    f32 = jnp.float32
    bf16 = jnp.bfloat16

    def xcopy(blk, slot):
        return pltpu.make_async_copy(
            x_hbm.at[pl.ds(pl.multiple_of(blk * TM, TM), TM), :], xbuf.at[slot], xsems.at[slot])

    def copies():
        return [
            pltpu.make_async_copy(wg_hbm.at[0:GA, :], wg_v.at[0:GA, :], sems.at[0]),
            pltpu.make_async_copy(wg_hbm.at[GA:DF, :], wg_v.at[GA:DF, :], sems.at[1]),
            pltpu.make_async_copy(wqkv_hbm, wqkv_raw, sems.at[2]),
            pltpu.make_async_copy(wu_hbm, wu_v, sems.at[3]),
            pltpu.make_async_copy(wo_hbm, wo_raw, sems.at[4]),
            pltpu.make_async_copy(wd_hbm, wd_v, sems.at[5]),
        ]

    def ln_stats(xb):
        x = xb.astype(f32)
        m = jnp.mean(x, axis=-1, keepdims=True)
        xc = x - m
        var = jnp.mean(xc * xc, axis=-1, keepdims=True)
        r = jax.lax.rsqrt(var + EPS)
        return m, r, (xc * r).astype(bf16)

    def prep_part(p):
        for j in range(4):
            tbuf[j, p * D:(p + 1) * D, :] = wqkv_raw[128 * j:128 * (j + 1), p * D:(p + 1) * D].astype(f32).T
        for j in range(4):
            for d in range(DH):
                rows = tbuf[j, pl.ds(p * D + d, H, stride=DH), :]
                wqkvT[p * D + d * H:p * D + (d + 1) * H, 128 * j:128 * (j + 1)] = rows.astype(bf16)

    def prep_wo():
        for j in range(4):
            tbuf2[j] = wo_raw[:, 128 * j:128 * (j + 1)].astype(f32)
        for j in range(4):
            for d in range(DH):
                wo_p[d * H:(d + 1) * H, 128 * j:128 * (j + 1)] = tbuf2[j, pl.ds(d, H, stride=DH), :].astype(bf16)

    def proj(lhs, p):
        return jax.lax.dot_general(lhs, wqkvT[p * D:(p + 1) * D, :], NT, preferred_element_type=f32)

    def store_part(y, p):
        for j in range(4):
            yj = y[:, 128 * j:128 * (j + 1)]
            if p == 0:
                qbuf[j] = yj * SCALE
            elif p == 1:
                kbuf[j, HALO:, :] = yj
            else:
                vbuf[j, HALO:, :] = yj

    def attention(first):
        for c in range(TM // RC):
            r0 = c * RC
            q = [qbuf[j, r0:r0 + RC, :] for j in range(4)]
            logits = []
            for w in range(W):
                s0 = HALO + r0 - DIL * w
                p = [q[j] * kbuf[j, s0:s0 + RC, :] for j in range(4)]
                p = (p[0] + p[1]) + (p[2] + p[3])
                p = p + pltpu.roll(p, 32, 1)
                p = p + pltpu.roll(p, 64, 1)
                if first and w > 0 and r0 < HALO:
                    row = r0 + jax.lax.broadcasted_iota(jnp.int32, (RC, 128), 0)
                    p = jnp.where(row >= DIL * w, p, NEG)
                logits.append(p)
            mx = logits[0]
            for w in range(1, W):
                mx = jnp.maximum(mx, logits[w])
            es = [jnp.exp2(l - mx) for l in logits]
            den = es[0]
            for w in range(1, W):
                den = den + es[w]
            inv = 1.0 / den
            for j in range(4):
                acc = None
                for w in range(W):
                    s0 = HALO + r0 - DIL * w
                    t = es[w] * vbuf[j, s0:s0 + RC, :]
                    acc = t if acc is None else acc + t
                obuf[r0:r0 + RC, 128 * j:128 * (j + 1)] = (acc * inv).astype(bf16)
        kbuf[:, 0:HALO, :] = kbuf[:, TM:TM + HALO, :]
        vbuf[:, 0:HALO, :] = vbuf[:, TM:TM + HALO, :]

    def geglu(g, u):
        gl = 0.5 * g * (1.0 + jnp.tanh(GELU_C * (g + 0.044715 * (g * g * g))))
        return (gl * u).astype(bf16)

    def tail(xb, h, prep=False):
        yb = jnp.dot(h, wd_v[...], preferred_element_type=f32)
        if prep:
            prep_wo()
        ya = jnp.dot(obuf[...], wo_p[...], preferred_element_type=f32)
        o_ref[...] = (xb.astype(f32) + ya + yb).astype(o_ref.dtype)

    def nt(lhs, w_ref, a, b):
        return jax.lax.dot_general(lhs, w_ref[a:b, :], NT, preferred_element_type=f32)

    @pl.when(i == 0)
    def _():
        xcopy(0, 0).start()
        cps = copies()
        cps[0].start()
        kbuf[:, 0:HALO, :] = jnp.zeros((4, HALO, 128), f32)
        vbuf[:, 0:HALO, :] = jnp.zeros((4, HALO, 128), f32)
        xcopy(0, 0).wait()
        cps[1].start()
        xb = xbuf[0]
        _, _, xn = ln_stats(xb)
        cps[0].wait()
        cps[2].start()
        g0 = nt(xn, wg_v, 0, GA)
        cps[1].wait()
        cps[3].start()
        g1 = nt(xn, wg_v, GA, GB)
        cps[2].wait()
        cps[4].start()
        cps[5].start()
        xcopy(1, 1).start()
        g2 = nt(xn, wg_v, GB, DF)
        for p in (1, 2, 0):
            prep_part(p)
            store_part(proj(xn, p), p)
        csbuf[...] = proj(jnp.ones((16, D), bf16), 1)
        cps[3].wait()
        cps[4].wait()
        cps[5].wait()
        u = nt(xn, wu_v, 0, DF)
        attention(True)
        g = jnp.concatenate([g0, g1, g2], axis=-1)
        tail(xb, geglu(g, u), True)

    @pl.when(i > 0)
    def _():
        slot = i % 2
        xcopy(i, slot).wait()

        @pl.when(i < NSTEP - 1)
        def _():
            xcopy(i + 1, 1 - slot).start()

        xb = xbuf[slot]
        kraw = proj(xb, 1)
        m, r, xn = ln_stats(xb)
        store_part(kraw * r - (r * m) * csbuf[0:1, :], 1)
        store_part(proj(xn, 2), 2)
        store_part(proj(xn, 0), 0)
        g = nt(xn, wg_v, 0, DF)
        u = nt(xn, wu_v, 0, DF)
        attention(False)
        tail(xb, geglu(g, u))


@jax.jit
def pallas_parallel_sum__sliding_local_dilated__glu_gated_geglu__prompt_kernel(
    A_x: jax.Array,
    A_wqkv: jax.Array,
    A_wo: jax.Array,
    B_x: jax.Array,
    B_w_gate: jax.Array,
    B_w_up: jax.Array,
    B_w_down: jax.Array,
):
    x = A_x.reshape(S, D)
    bf16 = jnp.bfloat16
    f32 = jnp.float32
    anyspec = pl.BlockSpec(memory_space=pl.ANY)
    out = pl.pallas_call(
        _kernel,
        grid=(NSTEP,),
        in_specs=[anyspec] * 6,
        out_specs=pl.BlockSpec((TM, D), lambda i: (i, 0)),
        out_shape=jax.ShapeDtypeStruct((S, D), bf16),
        scratch_shapes=[
            pltpu.VMEM((2, TM, D), bf16),
            pltpu.VMEM((D, 3 * D), bf16),
            pltpu.VMEM((D, D), bf16),
            pltpu.VMEM((DF, D), bf16),
            pltpu.VMEM((DF, D), bf16),
            pltpu.VMEM((DF, D), bf16),
            pltpu.VMEM((3 * D, D), bf16),
            pltpu.VMEM((D, D), bf16),
            pltpu.VMEM((4, 3 * D, 128), f32),
            pltpu.VMEM((4, D, 128), f32),
            pltpu.VMEM((16, D), f32),
            pltpu.VMEM((4, TM, 128), f32),
            pltpu.VMEM((4, TM + HALO, 128), f32),
            pltpu.VMEM((4, TM + HALO, 128), f32),
            pltpu.VMEM((TM, D), bf16),
            pltpu.SemaphoreType.DMA((6,)),
            pltpu.SemaphoreType.DMA((2,)),
        ],
        compiler_params=pltpu.CompilerParams(
            dimension_semantics=("arbitrary",),
            vmem_limit_bytes=100 * 1024 * 1024,
        ),
    )(x, A_wqkv, A_wo, B_w_gate.T, B_w_up.T, B_w_down)
    return out.reshape(1, S, D)
```

```python
import jax
import jax.numpy as jnp
import jax.experimental.pallas as pl
import jax.experimental.pallas.tpu as pltpu

S = 2048
D = 512
H = 32
DH = 16
W = 8
DIL = 2
DF = 1376
HALO = 16
TM = 512
NSTEP = S // TM
RC = 16
LC = 16
EPS = 1e-5
LOG2E = 1.4426950408889634
NEG = -1e9 * LOG2E
SCALE = DH ** -0.5 * LOG2E
GELU_C = 0.7978845608028654
NT = (((1,), (1,)), ((), ()))
PS = 17
PB = 552
GA, GB = 384, 1024


def _kernel(x_hbm, wqkv_hbm, wo_hbm, wg_hbm, wu_hbm, wd_hbm, o_ref,
            xbuf, wqkv_raw, wo_raw, wg_v, wu_v, wd_v, wqkvT, wo_p, tbuf, tbuf2,
            csbuf, qbuf, kbuf, vbuf, obuf, sems, xsems):
    i = pl.program_id(0)
    f32 = jnp.float32
    bf16 = jnp.bfloat16

    def xcopy(blk, slot):
        return pltpu.make_async_copy(
            x_hbm.at[pl.ds(pl.multiple_of(blk * TM, TM), TM), :], xbuf.at[slot], xsems.at[slot])

    def copies():
        return [
            pltpu.make_async_copy(wg_hbm.at[0:GA, :], wg_v.at[0:GA, :], sems.at[0]),
            pltpu.make_async_copy(wg_hbm.at[GA:DF, :], wg_v.at[GA:DF, :], sems.at[1]),
            pltpu.make_async_copy(wqkv_hbm, wqkv_raw, sems.at[2]),
            pltpu.make_async_copy(wu_hbm, wu_v, sems.at[3]),
            pltpu.make_async_copy(wo_hbm, wo_raw, sems.at[4]),
            pltpu.make_async_copy(wd_hbm, wd_v, sems.at[5]),
        ]

    def ln_stats(xref, lc):
        ms, rs, xns = [], [], []
        for c in range(TM // lc):
            x = xref[c * lc:(c + 1) * lc, :].astype(f32)
            m = jnp.mean(x, axis=-1, keepdims=True)
            xc = x - m
            var = jnp.mean(xc * xc, axis=-1, keepdims=True)
            r = jax.lax.rsqrt(var + EPS)
            ms.append(m)
            rs.append(r)
            xns.append((xc * r).astype(bf16))
        cat = lambda z: jnp.concatenate(z, axis=0)
        return cat(ms), cat(rs), cat(xns)

    def prep_part(p):
        for j in range(4):
            t = wqkv_raw[128 * j:128 * (j + 1), p * D:(p + 1) * D].astype(f32).T
            for h in range(H):
                tbuf[j, p * PB + h * PS:p * PB + h * PS + DH, :] = t[h * DH:(h + 1) * DH, :]
        for j in range(4):
            for d in range(DH):
                rows = tbuf[j, pl.ds(p * PB + d, H, stride=PS), :]
                wqkvT[p * D + d * H:p * D + (d + 1) * H, 128 * j:128 * (j + 1)] = rows.astype(bf16)

    def prep_wo():
        for j in range(4):
            t = wo_raw[:, 128 * j:128 * (j + 1)].astype(f32)
            for h in range(H):
                tbuf2[j, h * PS:h * PS + DH, :] = t[h * DH:(h + 1) * DH, :]
        for j in range(4):
            for d in range(DH):
                wo_p[d * H:(d + 1) * H, 128 * j:128 * (j + 1)] = (
                    tbuf2[j, pl.ds(d, H, stride=PS), :].astype(bf16))

    def proj(lhs, p):
        return jax.lax.dot_general(lhs, wqkvT[p * D:(p + 1) * D, :], NT, preferred_element_type=f32)

    def store_part(y, p):
        for j in range(4):
            yj = y[:, 128 * j:128 * (j + 1)]
            if p == 0:
                qbuf[j] = yj * SCALE
            elif p == 1:
                kbuf[j, HALO:, :] = yj
            else:
                vbuf[j, HALO:, :] = yj

    def attention(first):
        for c in range(TM // RC):
            r0 = c * RC
            q = [qbuf[j, r0:r0 + RC, :] for j in range(4)]
            logits = []
            for w in range(W):
                s0 = HALO + r0 - DIL * w
                p = [q[j] * kbuf[j, s0:s0 + RC, :] for j in range(4)]
                p = (p[0] + p[1]) + (p[2] + p[3])
                p = p + pltpu.roll(p, 32, 1)
                p = p + pltpu.roll(p, 64, 1)
                if first and w > 0 and r0 < HALO:
                    row = r0 + jax.lax.broadcasted_iota(jnp.int32, (RC, 128), 0)
                    p = jnp.where(row >= DIL * w, p, NEG)
                logits.append(p)
            mx = logits[0]
            for w in range(1, W):
                mx = jnp.maximum(mx, logits[w])
            es = [jnp.exp2(l - mx) for l in logits]
            den = es[0]
            for w in range(1, W):
                den = den + es[w]
            inv = 1.0 / den
            for j in range(4):
                acc = None
                for w in range(W):
                    s0 = HALO + r0 - DIL * w
                    t = es[w] * vbuf[j, s0:s0 + RC, :]
                    acc = t if acc is None else acc + t
                obuf[r0:r0 + RC, 128 * j:128 * (j + 1)] = (acc * inv).astype(bf16)
        kbuf[:, 0:HALO, :] = kbuf[:, TM:TM + HALO, :]
        vbuf[:, 0:HALO, :] = vbuf[:, TM:TM + HALO, :]

    def geglu(g, u):
        gl = 0.5 * g * (1.0 + jnp.tanh(GELU_C * (g + 0.044715 * (g * g * g))))
        return (gl * u).astype(bf16)

    def tail(xb, h, prep=False):
        yb = jnp.dot(h, wd_v[...], preferred_element_type=f32)
        if prep:
            prep_wo()
        ya = jnp.dot(obuf[...], wo_p[...], preferred_element_type=f32)
        o_ref[...] = ((xb.astype(f32) + yb) + ya).astype(o_ref.dtype)

    def nt(lhs, w_ref, a, b):
        return jax.lax.dot_general(lhs, w_ref[a:b, :], NT, preferred_element_type=f32)

    @pl.when(i == 0)
    def _():
        xcopy(0, 0).start()
        cps = copies()
        cps[0].start()
        kbuf[:, 0:HALO, :] = jnp.zeros((4, HALO, 128), f32)
        vbuf[:, 0:HALO, :] = jnp.zeros((4, HALO, 128), f32)
        xcopy(0, 0).wait()
        cps[1].start()
        xb = xbuf[0]
        _, _, xn = ln_stats(xbuf.at[0], TM)
        cps[0].wait()
        cps[2].start()
        g0 = nt(xn, wg_v, 0, GA)
        cps[1].wait()
        cps[3].start()
        g1 = nt(xn, wg_v, GA, GB)
        cps[2].wait()
        cps[4].start()
        cps[5].start()
        g2 = nt(xn, wg_v, GB, DF)
        for p in (1, 2):
            prep_part(p)
            store_part(proj(xn, p), p)
        csbuf[...] = proj(jnp.ones((16, D), bf16), 1)
        prep_part(0)
        cps[3].wait()
        cps[4].wait()
        cps[5].wait()
        xcopy(1, 1).start()
        store_part(proj(xn, 0), 0)
        u = nt(xn, wu_v, 0, DF)
        attention(True)
        g = jnp.concatenate([g0, g1, g2], axis=-1)
        tail(xb, geglu(g, u), True)

    @pl.when(i > 0)
    def _():
        slot = i % 2
        xcopy(i, slot).wait()

        @pl.when(i < NSTEP - 1)
        def _():
            xcopy(i + 1, 1 - slot).start()

        xb = xbuf[slot]
        kraw = proj(xb, 1)
        m, r, xn = ln_stats(xbuf.at[slot], LC)
        store_part(kraw * r - (r * m) * csbuf[0:1, :], 1)
        store_part(proj(xn, 2), 2)
        store_part(proj(xn, 0), 0)
        g = nt(xn, wg_v, 0, DF)
        u = nt(xn, wu_v, 0, DF)
        attention(False)
        tail(xb, geglu(g, u))


@jax.jit
def pallas_parallel_sum__sliding_local_dilated__glu_gated_geglu__prompt_kernel(
    A_x: jax.Array,
    A_wqkv: jax.Array,
    A_wo: jax.Array,
    B_x: jax.Array,
    B_w_gate: jax.Array,
    B_w_up: jax.Array,
    B_w_down: jax.Array,
):
    del B_x
    x = A_x.reshape(S, D)
    bf16 = jnp.bfloat16
    f32 = jnp.float32
    anyspec = pl.BlockSpec(memory_space=pl.ANY)
    out = pl.pallas_call(
        _kernel,
        grid=(NSTEP,),
        in_specs=[anyspec] * 6,
        out_specs=pl.BlockSpec((TM, D), lambda i: (i, 0)),
        out_shape=jax.ShapeDtypeStruct((S, D), bf16),
        scratch_shapes=[
            pltpu.VMEM((2, TM, D), bf16),
            pltpu.VMEM((D, 3 * D), bf16),
            pltpu.VMEM((D, D), bf16),
            pltpu.VMEM((DF, D), bf16),
            pltpu.VMEM((DF, D), bf16),
            pltpu.VMEM((DF, D), bf16),
            pltpu.VMEM((3 * D, D), bf16),
            pltpu.VMEM((D, D), bf16),
            pltpu.VMEM((4, 3 * PB, 128), f32),
            pltpu.VMEM((4, PB, 128), f32),
            pltpu.VMEM((16, D), f32),
            pltpu.VMEM((4, TM, 128), f32),
            pltpu.VMEM((4, TM + HALO, 128), f32),
            pltpu.VMEM((4, TM + HALO, 128), f32),
            pltpu.VMEM((TM, D), bf16),
            pltpu.SemaphoreType.DMA((6,)),
            pltpu.SemaphoreType.DMA((2,)),
        ],
        compiler_params=pltpu.CompilerParams(
            dimension_semantics=("arbitrary",),
            vmem_limit_bytes=100 * 1024 * 1024,
        ),
    )(x, A_wqkv, A_wo, B_w_gate.T, B_w_up.T, B_w_down)
    return out.reshape(1, S, D)
```
